```python
import os as _os
_os.environ.setdefault("JAX_PLATFORMS", "cpu")
import jax
import jax.numpy as jnp

def _softmax(x, axis=-1):
    return jax.nn.softmax(x, axis=axis)
def _gelu(x):
    return jax.nn.gelu(x, approximate=True)
def _silu(x):
    return jax.nn.silu(x)
def _sigmoid(x):
    return jax.nn.sigmoid(x)
def _layernorm(x, axis=-1, eps=1e-5):
    m = jnp.mean(x, axis=axis, keepdims=True)
    v = jnp.var(x, axis=axis, keepdims=True)
    return (x - m) / jnp.sqrt(v + eps)
def _scatter_add(tgt, idx, src, axis=0):
    return tgt.at[idx].add(src)
def _segment_sum(src, seg, n):
    return jax.ops.segment_sum(src, seg, n)
class _Rng:
    def __init__(self, key):
        self._k = key
    def _next(self):
        self._k, sub = jax.random.split(self._k)
        return sub
    def normal(self, shape):
        return jax.random.normal(self._next(), shape, dtype=jnp.bfloat16)
    def randint(self, lo, hi, shape):
        return jax.random.randint(self._next(), shape, lo, hi, dtype=jnp.int32)
    def uniform(self, shape, lo=0.0, hi=1.0):
        return jax.random.uniform(self._next(), shape, jnp.bfloat16, lo, hi)
    def permutation(self, n):
        return jax.random.permutation(self._next(), n)


kernel_name = 'parallel_sum__sliding_local_dilated__dense_activation_mish__prompt'

def setup_inputs():
    _rng = _Rng(jax.random.key(int.from_bytes(__import__("os").urandom(4), "little")))
    _w = (lambda a: (lambda t: t.astype(jnp.bfloat16) if jnp.issubdtype(t.dtype, jnp.floating) else t)(jnp.asarray(a)))
    def _A_setup():
        B, S, D = 1, 2048, 576
        return {
            "x": _w((lambda *s: _rng.normal(s) * 0.05)(B, S, D)),
            "wqkv": _w((lambda *s: _rng.normal(s) * 0.05)(D, 3 * D)),
            "wo": _w((lambda *s: _rng.normal(s) * 0.05)(D, D)),
        }
    _A_in = _A_setup()

    def _B_setup():
        B, S, D, F = 1, 2048, 576, 4608
        return {
            "x": _w((lambda *s: _rng.normal(s) * 0.05)(B, S, D)),
            "w1": _w((lambda *s: _rng.normal(s) * 1.6)(D, F) * (D ** -0.5)),
            "b1": _w((lambda *s: _rng.normal(s) * 0.2)(F)),
            "w2": _w((lambda *s: _rng.normal(s) * 0.2)(F, D) * (F ** -0.5)),
        }
    _B_in = _B_setup()

    return {
        "A_x": _A_in["x"],
        "A_wqkv": _A_in["wqkv"],
        "A_wo": _A_in["wo"],
        "B_x": _B_in["x"],
        "B_w1": _B_in["w1"],
        "B_b1": _B_in["b1"],
        "B_w2": _B_in["w2"],
    }

def reference(A_x, A_wqkv, A_wo, B_x, B_w1, B_b1, B_w2):
    def _A_ref(x, wqkv, wo):
        B, S, D = x.shape
        H = 32; Dh = D // H
        W, dil = 8, 2
        qkv = (lambda x, *d: x.transpose(*d))((x @ wqkv).reshape(B, S, 3, H, Dh), 2, 0, 3, 1, 4)
        q, k, v = qkv[0], qkv[1], qkv[2]
        scale = Dh ** -0.5
        pos = jnp.arange(S)
        off = jnp.arange(W) * dil
        idx = pos[:, None] - off[None, :]
        mask = idx >= 0
        idx_c = jnp.where(mask, idx, 0).reshape(-1)
        kg = k[:, :, idx_c, :].reshape(B, H, S, W, Dh)
        vg = v[:, :, idx_c, :].reshape(B, H, S, W, Dh)
        logits = jnp.einsum("bhsd,bhswd->bhsw", q, kg) * scale
        logits = jnp.where(mask[None, None, :, :], logits, -1e9)
        attn = _softmax(logits, axis=-1)
        o = jnp.einsum("bhsw,bhswd->bhsd", attn, vg)
        return (lambda x, *d: x.transpose(*d))(o, 0, 2, 1, 3).reshape(B, S, D) @ wo

    def _B_ref(x, w1, b1, w2):
        h = jnp.einsum("bsd,df->bsf", x, w1) + b1
        sp = jnp.log1p(jnp.exp(-jnp.abs(h))) + jnp.where(h > 0, h, jnp.zeros_like(h))
        act = h * jnp.tanh(sp)
        return jnp.einsum("bsf,fd->bsd", act, w2)

    x = A_x
    xn = _layernorm(x, axis=-1)
    return x + _A_ref(xn, A_wqkv, A_wo) + _B_ref(xn, B_w1, B_b1, B_w2)
```

```python
import jax
import jax.numpy as jnp
import numpy as np
import jax.experimental.pallas as pl
import jax.experimental.pallas.tpu as pltpu

S, D, F = 2048, 576, 4608
H, DH, W, DIL = 32, 18, 8, 2
TM, TF = 256, 512
NS, NC = S // TM, F // TF
NRB = TM // 8
NP = 1792
HALO = 16
NT = (((1,), (1,)), ((), ()))
LOG2E = 1.4426950408889634
QSCALE = (DH ** -0.5) * LOG2E
QBITS = int(np.float32(QSCALE).view(np.int32))
NEG = -1e9 * LOG2E
SCHED_A = [[0, 1, 2, 3], [3], [3], [3], [3], [3], [], []]
SCHED_R = [[0, 1, 2, 3], [0, 1, 2, 3], [0, 1, 2, 3], [0, 1, 2, 3], [0, 1, 2, 3], [0, 1, 2], []]
LN1 = 2
LNT = 0
f32, bf16, u32, i32 = jnp.float32, jnp.bfloat16, jnp.uint32, jnp.int32


def mish(h):
    e = jnp.exp(jnp.minimum(h, 20.0))
    n = e * (e + 2.0)
    return h * (n * pl.reciprocal(n + 2.0, approx=True))


def fold8(a):
    n = a.shape[0] // 8
    parts = [a[8 * i:8 * i + 8] for i in range(n)]
    while len(parts) > 1:
        nxt = [parts[i] + parts[i + 1] for i in range(0, len(parts) - 1, 2)]
        if len(parts) % 2:
            nxt.append(parts[-1])
        parts = nxt
    return parts[0]


def const_from(tok, bits):
    t = pltpu.bitcast(tok, i32)
    return pltpu.bitcast(jnp.minimum(jnp.maximum(t, bits), bits), f32)


def kern(x_hbm, wqkv_hbm, wo_hbm, w1_hbm, b1_hbm, w2_hbm, out_hbm,
         x_buf, out_buf, w_buf, wqkv_buf, wo_buf, b1_buf, b1f,
         xn_buf, acc, act_last, q_scr, kv_scr, o_scr, t_scr, t2_scr, wpt, wot, sem):
    def cx(s, k):
        return pltpu.make_async_copy(x_hbm.at[:, s * TM:(s + 1) * TM], x_buf.at[s], sem.at[k])
    def wx(s0, s1, k):
        pltpu.make_async_copy(x_buf.at[s0:s1], x_buf.at[s0:s1], sem.at[k]).wait()
    def cw1(c, k):
        return pltpu.make_async_copy(w1_hbm.at[:, c * TF:(c + 1) * TF], w_buf.at[c, 0], sem.at[k])
    def cw2(c, k):
        return pltpu.make_async_copy(w2_hbm.at[:, c * TF:(c + 1) * TF], w_buf.at[c, 1], sem.at[k])
    def ww(c0, c1, k):
        pltpu.make_async_copy(w_buf.at[c0:c1], w_buf.at[c0:c1], sem.at[k]).wait()
    cqkv = pltpu.make_async_copy(wqkv_hbm, wqkv_buf, sem.at[7])
    cwo = pltpu.make_async_copy(wo_hbm, wo_buf, sem.at[8])
    cb1 = pltpu.make_async_copy(b1_hbm, b1_buf, sem.at[9])
    def cout(s):
        return pltpu.make_async_copy(out_buf.at[s], out_hbm.at[:, s * TM:(s + 1) * TM], sem.at[12])

    def ln(s):
        tot = None
        for r in range(0, D, 64):
            p = fold8(x_buf[s, r:r + 64, :].astype(f32))
            tot = p if tot is None else tot + p
        m = jnp.sum(tot, axis=0, keepdims=True) * (1.0 / D)
        tot = None
        for r in range(0, D, 96):
            d = x_buf[s, r:r + 96, :].astype(f32) - m
            p = fold8(d * d)
            tot = p if tot is None else tot + p
        v = jnp.sum(tot, axis=0, keepdims=True) * (1.0 / D)
        rs = jax.lax.rsqrt(v + 1e-5)
        for r in range(0, D, 128):
            n = min(128, D - r)
            blk = (x_buf[s, r:r + n, :].astype(f32) - m) * rs
            xn_buf[s, :, r:r + n] = pltpu.bitcast(blk.astype(bf16).T, u32)

    def zf_from(tok):
        t = pltpu.bitcast(tok, i32)
        return pltpu.bitcast(jnp.minimum(jnp.maximum(t, 0), 0), f32)

    def ln_c(s, LNC=3):
        tot = None
        for r in range(0, D, 64):
            blk = x_buf[s, r:r + 64, :].astype(f32)
            for g in range(8):
                p = blk[8 * g:8 * g + 8]
                tot = p if tot is None else tot + p
        m = jnp.broadcast_to(jnp.sum(tot, axis=0, keepdims=True) * (1.0 / D), (8, TM))
        tots = []
        for hh in range(2):
            mh = m[:, hh * 128:(hh + 1) * 128]
            if hh == 1 and LNC >= 2:
                mh = mh + zf_from(tots[0])
            tot = None
            for r in range(0, D, 96):
                d = x_buf[s, r:r + 96, hh * 128:(hh + 1) * 128].astype(f32).reshape(12, 8, 128) - mh[None]
                dd = d * d
                for g in range(12):
                    tot = dd[g] if tot is None else tot + dd[g]
            tots.append(tot)
        v = jnp.sum(jnp.concatenate(tots, axis=1), axis=0, keepdims=True) * (1.0 / D)
        rs = jnp.broadcast_to(jax.lax.rsqrt(v + 1e-5), (8, TM))
        tok = None
        for r in range(0, D, 128):
            n = min(128, D - r)
            mk = m
            if tok is not None and LNC >= 3:
                z = zf_from(tok)
                mk = m + jnp.concatenate([z, z], axis=1)
            blk = (x_buf[s, r:r + n, :].astype(f32).reshape(n // 8, 8, TM) - mk[None]) * rs[None]
            t = pltpu.bitcast(blk.reshape(n, TM).astype(bf16).T, u32)
            xn_buf[s, :, r:r + n] = t
            if n == 128:
                tok = t[LNT:LNT + 8, :]

    def load_xn(s):
        return pltpu.bitcast(xn_buf[s], bf16)

    def mm1(c, s):
        h = jnp.dot(load_xn(s), w_buf[c, 0], preferred_element_type=f32) + b1f[c]
        return mish(h).astype(bf16)

    def mm2(c, a):
        return jax.lax.dot_general(w_buf[c, 1], a, NT, preferred_element_type=f32)

    def toks_a(a):
        u = pltpu.bitcast(a, u32)
        return [u[120:128, 128:256], u[120:128, 384:512]]

    def toks_r(r):
        return [r[568:576, 0:128], r[568:576, 128:256]]

    def qkv_mm(j):
        kv_scr[:, 0:HALO, :] = kv_scr[:, TM:TM + HALO, :]
        xn = load_xn(j)
        for g in range(7):
            wblk = pltpu.bitcast(wpt[g * 128:(g + 1) * 128, :], bf16)
            r = jax.lax.dot_general(xn, wblk, NT, preferred_element_type=f32)
            for hh in range(2):
                t = 2 * g + hh
                blk = r[:, hh * 128:(hh + 1) * 128]
                if t < 4:
                    q_scr[t] = blk
                elif t < 12:
                    kv_scr[t - 4, HALO:HALO + TM, :] = blk
                elif t == 12:
                    q_scr[4] = blk
                else:
                    kv_scr[8, HALO:HALO + TM, :] = blk

    def attn_rb(j, r0, tok):
        sc = const_from(tok, QBITS)
        q = [q_scr[t, pl.ds(r0, 8, stride=2), :] * sc for t in range(5)]
        def kv(t, w):
            return kv_scr[t, pl.ds(HALO + r0 - DIL * w, 8, stride=2), :]
        ls = []
        for w in range(W):
            p = q[0] * kv(0, w)
            for t in range(1, 4):
                p = p + q[t] * kv(t, w)
            p = p + q[4] * kv(8, w)
            p = p + pltpu.roll(p, 64, 1)
            p = p + pltpu.roll(p, 32, 1)
            if r0 < 16 and w > 0:
                pos = j * TM + r0 + 2 * jax.lax.broadcasted_iota(jnp.int32, (8, 128), 0)
                p = jnp.where(pos >= DIL * w, p, NEG)
            ls.append(p)
        mx = jnp.maximum(jnp.maximum(jnp.maximum(ls[0], ls[1]), jnp.maximum(ls[2], ls[3])),
                         jnp.maximum(jnp.maximum(ls[4], ls[5]), jnp.maximum(ls[6], ls[7])))
        ps = [jnp.exp2(l - mx) for l in ls]
        den = ((ps[0] + ps[1]) + (ps[2] + ps[3])) + ((ps[4] + ps[5]) + (ps[6] + ps[7]))
        r = pl.reciprocal(den, approx=True)
        outs = []
        for t in (4, 5, 6, 7, 8):
            a = None
            for w in range(W):
                u = ps[w] * kv(t, w)
                a = u if a is None else a + u
            outs.append(a * r)
        return outs

    def attn_pair(j, p2, toks):
        a = attn_rb(j, 16 * p2, toks[0]); b = attn_rb(j, 16 * p2 + 1, toks[1])
        for t in range(5):
            o_scr[p2 * 8:(p2 + 1) * 8, t * 128:(t + 1) * 128] = pltpu.pack_elementwise([a[t], b[t]], packed_dtype=bf16)

    def wo_mm():
        return jax.lax.dot_general(pltpu.bitcast(wot[...], bf16), pltpu.bitcast(o_scr[...], bf16), NT,
                                   preferred_element_type=f32)

    def zero_from(tok):
        t = pltpu.bitcast(tok, i32)
        return pltpu.bitcast(jnp.minimum(jnp.maximum(t, 0), 0), u32)

    def gate(x, z):
        u = pltpu.bitcast(x, u32)
        k, n = u.shape
        return (u.reshape(k // 8, 8, n) | z[None, :, :n]).reshape(k, n)

    def prep_qkv_t(nb, tok):
        z = zero_from(tok)
        nc = 128 if nb < 13 else 64
        for cb in range(5):
            kc = 128 if cb < 4 else 64
            blk = pltpu.bitcast(gate(wqkv_buf[cb * 128:cb * 128 + kc, nb * 128:nb * 128 + nc], z), bf16)
            t = blk.T.astype(f32)
            if kc < 128:
                t = jnp.concatenate([t, jnp.zeros((nc, 128 - kc), f32)], axis=1)
            t_scr[cb, nb * 128:nb * 128 + nc, :] = t

    def prep_qkv_g(t, d, tok):
        z = zero_from(tok)
        if d < 16:
            row = t * 512 + d * 32
        else:
            row = (1536, 1664, 1728)[t] + (d - 16) * 32
        st = t * D + d
        for cb in range(5):
            kc = 128 if cb < 4 else 64
            ev = t_scr[cb, pl.ds(st, 16, stride=2 * DH), :]
            od = t_scr[cb, pl.ds(st + DH, 16, stride=2 * DH), :]
            pk = pltpu.pack_elementwise([pltpu.bitcast(gate(ev, z), f32), od], packed_dtype=bf16)
            wpt[row // 2:row // 2 + 16, cb * 128:cb * 128 + kc] = pk[:, :kc]

    def prep_wo_s(cb, tok):
        z = zero_from(tok)
        kc = 128 if cb < 4 else 64
        t = pltpu.bitcast(gate(wo_buf[:, cb * 128:cb * 128 + kc], z), bf16).astype(f32)
        if kc < 128:
            t = jnp.concatenate([t, jnp.zeros((D, 128 - kc), f32)], axis=1)
        t2_scr[cb] = t

    def prep_wo_g(kb, tok):
        z = zero_from(tok)
        for cb in range(5):
            kc = 128 if cb < 4 else 64
            g = lambda d: t2_scr[cb, pl.ds(d, H, stride=DH), :]
            if kb < 4:
                rows = [pltpu.bitcast(gate(g(kb * 4 + dd), z), f32) for dd in range(4)]
            else:
                rows = [jnp.zeros((64, 128), f32)] + [pltpu.bitcast(gate(g(dd), z), f32) for dd in (16, 17)]
            blk = jnp.concatenate(rows, axis=0).astype(bf16).T
            wot[cb * 64:cb * 64 + kc // 2, kb * 128:(kb + 1) * 128] = pltpu.bitcast(blk[:kc], u32)

    def tk_a(a):
        u = pltpu.bitcast(a, u32)
        return [u[120:128, n * 128:(n + 1) * 128] for n in range(4)]

    def tk_r(r):
        return [r[rows:rows + 8, n * 128:(n + 1) * 128] for n in range(2) for rows in (280, 568)]

    def mm1h(s, hh):
        h = jnp.dot(load_xn(s), w_buf[0, 0, :, hh * 256:(hh + 1) * 256], preferred_element_type=f32) + b1f[0, :, hh * 256:(hh + 1) * 256]
        return mish(h).astype(bf16)

    def ch(hh, k):
        return pltpu.make_async_copy(w1_hbm.at[:, hh * 256:(hh + 1) * 256], w_buf.at[0, 0, :, hh * 256:(hh + 1) * 256], sem.at[k])

    def res(s):
        return x_buf[s].astype(f32)

    cx(0, 0).start(); ch(0, 1).start(); cb1.start(); cx(1, 2).start()
    kv_scr[:, TM:TM + HALO, :] = jnp.zeros((9, HALO, 128), f32)
    wpt[800:832, :] = jnp.zeros((32, D), u32)
    cx(0, 0).wait()
    ch(1, 13).start(); cw2(0, 3).start()
    ln(0)
    ch(0, 1).wait(); cb1.wait()
    cx(2, 4).start(); cx(3, 5).start(); cx(4, 5).start()
    for c in range(NC):
        b1f[c] = b1_buf[c * TF:(c + 1) * TF].astype(f32)[None, :]
    a0a = mm1h(0, 0)
    cx(1, 2).wait(); ch(1, 13).wait()
    cx(5, 5).start(); cqkv.start()
    a0b = mm1h(0, 1)
    a0 = jnp.concatenate([a0a, a0b], axis=1)
    ln_c(1, LN1)
    a1 = mm1(0, 1)
    cw2(0, 3).wait(); cx(2, 4).wait()
    cx(6, 6).start(); cx(7, 6).start(); cwo.start()
    acc[0] = mm2(0, a0) + res(0)
    ln_c(2)
    a2 = mm1(0, 2)
    acc[1] = mm2(0, a1) + res(1)
    wx(3, 6, 5)
    cw1(1, 10).start(); cw2(1, 10).start()
    acc[2] = mm2(0, a2) + res(2)
    ln_c(3)
    a3 = mm1(0, 3)
    ln_c(4)
    a4 = mm1(0, 4)
    ln_c(5)
    acc[3] = mm2(0, a3) + res(3)
    cqkv.wait(); wx(6, 8, 6); cwo.wait()
    for c in range(2, NC):
        cw1(c, 11).start(); cw2(c, 11).start()
    a5 = mm1(0, 5)
    tk = tk_a(a5)
    for k in range(4):
        prep_qkv_t(2 * k, tk[k]); prep_qkv_t(2 * k + 1, tk[k])
    ln_c(6)
    r = mm2(0, a4) + res(4)
    acc[4] = r
    tk = tk_r(r)
    for k in range(3):
        prep_qkv_t(8 + 2 * k, tk[k]); prep_qkv_t(9 + 2 * k, tk[k])
    for cb in range(5):
        prep_wo_s(cb, tk[3 if cb > 1 else 2])
    a6 = mm1(0, 6)
    ln_c(7)
    tk = tk_a(a6)
    for d in range(DH):
        prep_qkv_g(0, d, tk[d * 4 // DH])
    r = mm2(0, a5) + res(5)
    acc[5] = r
    tk = tk_r(r)
    for d in range(DH):
        prep_qkv_g(1, d, tk[d * 2 // DH])
    for kb in range(5):
        prep_wo_g(kb, tk[2 if kb < 3 else 3])
    a7 = mm1(0, 7)
    tk = tk_a(a7)
    for d in range(DH):
        prep_qkv_g(2, d, tk[d * 3 // DH])
    acc[6] = mm2(0, a6) + res(6)
    act_last[...] = pltpu.bitcast(a7, u32)
    acc[NS - 1] = res(NS - 1)
    ww(1, 2, 10)

    def body(cc, carry):
        c = cc
        j = c - 1
        @pl.when(cc == 2)
        def _():
            ww(2, NC, 11)
        acc[NS - 1] = acc[NS - 1] + mm2(c - 1, pltpu.bitcast(act_last[...], bf16))
        qkv_mm(j)
        prev = None
        toks = []
        tnow = 0
        pend = []
        rb_done = 0
        outs = {}
        def run_rb(i, tok):
            outs[i] = attn_rb(j, 16 * (i // 2) + (i % 2), tok)
            if i % 2 == 1:
                p2 = i // 2
                for t in range(5):
                    o_scr[p2 * 8:(p2 + 1) * 8, t * 128:(t + 1) * 128] = pltpu.pack_elementwise(
                        [outs[i - 1][t], outs[i][t]], packed_dtype=bf16)
        i = 0
        for s in range(NS):
            a = mm1(c, s)
            u = pltpu.bitcast(a, u32)
            for n in SCHED_A[s]:
                run_rb(i, u[120:128, n * 128:(n + 1) * 128]); i += 1
            if prev is not None:
                r = acc[s - 1] + mm2(c, prev)
                acc[s - 1] = r
                out_buf[s - 1] = r.astype(bf16)
                @pl.when(c == NC - 1)
                def _():
                    cout(s - 1).start()
                for n in SCHED_R[s - 1]:
                    rows = (280, 568)[n % 2]
                    run_rb(i, r[rows:rows + 8, (n // 2) * 128:(n // 2 + 1) * 128]); i += 1
            prev = a
        assert i == 32, i
        acc[j] = acc[j] + wo_mm()
        act_last[...] = pltpu.bitcast(prev, u32)
        return carry
    jax.lax.fori_loop(1, NC, body, 0)
    r = acc[NS - 1] + mm2(NC - 1, pltpu.bitcast(act_last[...], bf16))
    out_buf[NS - 1] = r.astype(bf16)
    cout(NS - 1).start()
    pltpu.make_async_copy(out_buf, out_buf, sem.at[12]).wait()


@jax.jit
def pallas_parallel_sum__sliding_local_dilated__dense_activation_mish__prompt_kernel(
        A_x, A_wqkv, A_wo, B_x, B_w1, B_b1, B_w2):
    xt = A_x.reshape(S, D).T
    any_spec = pl.BlockSpec(memory_space=pl.ANY)
    ot = pl.pallas_call(
        kern,
        in_specs=[any_spec] * 6,
        out_specs=any_spec,
        out_shape=jax.ShapeDtypeStruct((D, S), bf16),
        scratch_shapes=[
            pltpu.VMEM((NS, D, TM), bf16),
            pltpu.VMEM((NS, D, TM), bf16),
            pltpu.VMEM((NC, 2, D, TF), bf16),
            pltpu.VMEM((D, 3 * D), bf16),
            pltpu.VMEM((D, D), bf16),
            pltpu.VMEM((F,), bf16),
            pltpu.VMEM((NC, 1, TF), f32),
            pltpu.VMEM((NS, TM // 2, D), u32),
            pltpu.VMEM((NS, D, TM), f32),
            pltpu.VMEM((TM // 2, TF), u32),
            pltpu.VMEM((5, TM, 128), f32),
            pltpu.VMEM((9, TM + HALO, 128), f32),
            pltpu.VMEM((TM // 2, 640), u32),
            pltpu.VMEM((5, 3 * D, 128), f32),
            pltpu.VMEM((5, D, 128), f32),
            pltpu.VMEM((NP // 2, D), u32),
            pltpu.VMEM((D // 2, 640), u32),
            pltpu.SemaphoreType.DMA((16,)),
        ],
        compiler_params=pltpu.CompilerParams(vmem_limit_bytes=100 * 1024 * 1024),
    )(xt, A_wqkv, A_wo, B_w1, B_b1, B_w2.T)
    return ot.T.reshape(1, S, D)
```

```python
import jax
import jax.numpy as jnp
import numpy as np
import jax.experimental.pallas as pl
import jax.experimental.pallas.tpu as pltpu

S, D, F = 2048, 576, 4608
H, DH, W, DIL = 32, 18, 8, 2
TM, TF = 256, 512
NS, NC = S // TM, F // TF
NRB = TM // 8
NP = 1792
HALO = 16
NT = (((1,), (1,)), ((), ()))
LOG2E = 1.4426950408889634
QSCALE = (DH ** -0.5) * LOG2E
QBITS = int(np.float32(QSCALE).view(np.int32))
NEG = -1e9 * LOG2E
SCHED_A = [[0, 1, 2, 3], [3], [3], [3], [3], [3], [], []]
SCHED_R = [[0, 1, 2, 3], [0, 1, 2, 3], [0, 1, 2, 3], [0, 1, 2, 3], [0, 1, 2, 3], [0, 1, 2], []]
LN1 = 2
LNT = 0
QORDER = (1, 2, 0)
ESPLIT = {0: [(0, D, 0), (0, D, 1)], 1: [(0, D, 0), (0, 288, 1), (288, D, 1)], 2: [(0, D, 0), (0, 384, 1), (384, D, 1)], 3: [(0, D, 0), (0, 448, 1), (448, D, 1)]}[1]
NSPLIT = 128
M2S = 0
QS = 0
WS = 0
L7T = 0
f32, bf16, u32, i32 = jnp.float32, jnp.bfloat16, jnp.uint32, jnp.int32


def mish(h):
    e = jnp.exp(jnp.minimum(h, 20.0))
    n = e * (e + 2.0)
    return h * (n * pl.reciprocal(n + 2.0, approx=True))


def fold8(a):
    n = a.shape[0] // 8
    parts = [a[8 * i:8 * i + 8] for i in range(n)]
    while len(parts) > 1:
        nxt = [parts[i] + parts[i + 1] for i in range(0, len(parts) - 1, 2)]
        if len(parts) % 2:
            nxt.append(parts[-1])
        parts = nxt
    return parts[0]


def const_from(tok, bits):
    t = pltpu.bitcast(tok, i32)
    return pltpu.bitcast(jnp.minimum(jnp.maximum(t, bits), bits), f32)


def kern(x_hbm, wqkv_hbm, wo_hbm, w1_hbm, b1_hbm, w2_hbm, out_hbm,
         x_buf, out_buf, w_buf, wqkv_buf, wo_buf, b1_buf, b1f,
         xn_buf, st_buf, acc, act_last, q_scr, kv_scr, o_scr, t_scr, t2_scr, wot, sem):
    def cx(s, k):
        return pltpu.make_async_copy(x_hbm.at[:, s * TM:(s + 1) * TM], x_buf.at[s], sem.at[k])
    def wx(s0, s1, k):
        pltpu.make_async_copy(x_buf.at[s0:s1], x_buf.at[s0:s1], sem.at[k]).wait()
    def cw1(c, k):
        return pltpu.make_async_copy(w1_hbm.at[:, c * TF:(c + 1) * TF], w_buf.at[c, 0], sem.at[k])
    def cw2(c, k):
        return pltpu.make_async_copy(w2_hbm.at[:, c * TF:(c + 1) * TF], w_buf.at[c, 1], sem.at[k])
    def ww(c0, c1, k):
        pltpu.make_async_copy(w_buf.at[c0:c1], w_buf.at[c0:c1], sem.at[k]).wait()
    cqkv = pltpu.make_async_copy(wqkv_hbm, wqkv_buf, sem.at[2])
    cwo = pltpu.make_async_copy(wo_hbm, wo_buf, sem.at[2])
    cb1 = pltpu.make_async_copy(b1_hbm, b1_buf, sem.at[1])
    def cout(s):
        return pltpu.make_async_copy(out_buf.at[s], out_hbm.at[:, s * TM:(s + 1) * TM], sem.at[2])

    def ln(s):
        tot = None
        for r in range(0, D, 64):
            p = fold8(x_buf[s, r:r + 64, :].astype(f32))
            tot = p if tot is None else tot + p
        m = jnp.sum(tot, axis=0, keepdims=True) * (1.0 / D)
        tot = None
        for r in range(0, D, 96):
            d = x_buf[s, r:r + 96, :].astype(f32) - m
            p = fold8(d * d)
            tot = p if tot is None else tot + p
        v = jnp.sum(tot, axis=0, keepdims=True) * (1.0 / D)
        rs = jax.lax.rsqrt(v + 1e-5)
        st_buf[s, 0] = jnp.broadcast_to(m, (8, TM))
        st_buf[s, 1] = jnp.broadcast_to(rs, (8, TM))
        for r in range(0, D, 128):
            n = min(128, D - r)
            blk = ((x_buf[s, r:r + n, :].astype(f32) - m) * rs).astype(bf16)
            xn_buf[s, :, r:r + n] = pltpu.bitcast(blk.T, u32)

    def zf_from(tok):
        t = pltpu.bitcast(tok, i32)
        return pltpu.bitcast(jnp.minimum(jnp.maximum(t, 0), 0), f32)

    def ln_c(s, LNC=3, tok0=None):
        tot = None
        if tok0 is not None:
            z0 = zf_from(tok0)
            tot = jnp.concatenate([z0, z0], axis=1)
        for r in range(0, D, 64):
            blk = x_buf[s, r:r + 64, :].astype(f32)
            for g in range(8):
                p = blk[8 * g:8 * g + 8]
                tot = p if tot is None else tot + p
        m = jnp.broadcast_to(jnp.sum(tot, axis=0, keepdims=True) * (1.0 / D), (8, TM))
        tots = []
        for hh in range(2):
            mh = m[:, hh * 128:(hh + 1) * 128]
            if hh == 1 and LNC >= 2:
                mh = mh + zf_from(tots[0])
            tot = None
            for r in range(0, D, 96):
                d = x_buf[s, r:r + 96, hh * 128:(hh + 1) * 128].astype(f32).reshape(12, 8, 128) - mh[None]
                dd = d * d
                for g in range(12):
                    tot = dd[g] if tot is None else tot + dd[g]
            tots.append(tot)
        v = jnp.sum(jnp.concatenate(tots, axis=1), axis=0, keepdims=True) * (1.0 / D)
        rs = jnp.broadcast_to(jax.lax.rsqrt(v + 1e-5), (8, TM))
        st_buf[s, 0] = m
        st_buf[s, 1] = rs
        tok = None
        for r in range(0, D, 128):
            n = min(128, D - r)
            mk = m
            if tok is not None and LNC >= 3:
                z = zf_from(tok)
                mk = m + jnp.concatenate([z, z], axis=1)
            blk = (x_buf[s, r:r + n, :].astype(f32).reshape(n // 8, 8, TM) - mk[None]) * rs[None]
            blk = blk.reshape(n, TM).astype(bf16)
            t = pltpu.bitcast(blk.T, u32)
            xn_buf[s, :, r:r + n] = t
            if n == 128:
                tok = t[LNT:LNT + 8, :]

    def load_xn(s):
        return pltpu.bitcast(xn_buf[s], bf16)

    def mm1(c, s):
        outs = []
        for n0 in range(0, TF, NSPLIT):
            h = jnp.dot(load_xn(s), w_buf[c, 0, :, n0:n0 + NSPLIT], preferred_element_type=f32) + b1f[c, :, n0:n0 + NSPLIT]
            outs.append(mish(h).astype(bf16))
        return outs[0] if len(outs) == 1 else jnp.concatenate(outs, axis=1)

    def mm2(c, a):
        if M2S:
            return jnp.concatenate([jax.lax.dot_general(w_buf[c, 1], a[hh * 128:(hh + 1) * 128], NT, preferred_element_type=f32) for hh in range(2)], axis=1)
        return jax.lax.dot_general(w_buf[c, 1], a, NT, preferred_element_type=f32)

    def toks_a(a):
        u = pltpu.bitcast(a, u32)
        return [u[120:128, 128:256], u[120:128, 384:512]]

    def toks_r(r):
        return [r[568:576, 0:128], r[568:576, 128:256]]

    def qkv_mm(j):
        kv_scr[:, 0:HALO, :] = kv_scr[:, TM:TM + HALO, :]
        xnt = ((x_buf[j].astype(f32).reshape(D // 8, 8, TM) - st_buf[j, 0][None]) * st_buf[j, 1][None]
               ).reshape(D, TM).astype(bf16)
        tails = []
        for t in QORDER:
            cols = []
            for cb in range(5):
                col = jnp.concatenate([t_scr[cb, pl.ds(t * (D // 2) + dp, H, stride=DH // 2), :] for dp in range(DH // 2)], axis=0)
                cols.append(col if cb < 4 else col[:, :64])
            wblk = pltpu.bitcast(jnp.concatenate(cols, axis=1), bf16)
            if QS:
                r = jnp.concatenate([jnp.dot(wblk, xnt[:, hh * 128:(hh + 1) * 128], preferred_element_type=f32) for hh in range(2)], axis=1)
            else:
                r = jnp.dot(wblk, xnt, preferred_element_type=f32)
            for g in range(4):
                blk = r[g * 128:(g + 1) * 128].T
                if t == 0:
                    q_scr[g] = blk
                else:
                    kv_scr[(t - 1) * 4 + g, HALO:HALO + TM, :] = blk
            if t == 0:
                q_scr[4] = jnp.concatenate([r[512:576], jnp.zeros((64, TM), f32)], axis=0).T
            else:
                tails.append(r[512:576])
        kv_scr[8, HALO:HALO + TM, :] = jnp.concatenate(tails, axis=0).T

    def attn_rb(j, r0, tok):
        sc = const_from(tok, QBITS)
        odd = (jax.lax.broadcasted_iota(jnp.int32, (8, 128), 1) & 1) == 1
        q = [q_scr[t, r0:r0 + 8, :] * sc for t in range(5)]
        def kv(t, w):
            return kv_scr[t, pl.ds(HALO + r0 - DIL * w, 8), :]
        ls = []
        for w in range(W):
            p = q[0] * kv(0, w)
            for t in range(1, 4):
                p = p + q[t] * kv(t, w)
            p = p + q[4] * kv(8, w)
            p = p + pltpu.roll(p, 64, 1)
            p = p + jnp.where(odd, pltpu.roll(p, 1, 1), pltpu.roll(p, 127, 1))
            if r0 < 16 and w > 0:
                pos = j * TM + r0 + jax.lax.broadcasted_iota(jnp.int32, (8, 128), 0)
                p = jnp.where(pos >= DIL * w, p, NEG)
            ls.append(p)
        mx = jnp.maximum(jnp.maximum(jnp.maximum(ls[0], ls[1]), jnp.maximum(ls[2], ls[3])),
                         jnp.maximum(jnp.maximum(ls[4], ls[5]), jnp.maximum(ls[6], ls[7])))
        ps = [jnp.exp2(l - mx) for l in ls]
        den = ((ps[0] + ps[1]) + (ps[2] + ps[3])) + ((ps[4] + ps[5]) + (ps[6] + ps[7]))
        r = pl.reciprocal(den, approx=True)
        outs = []
        for t in (4, 5, 6, 7, 8):
            a = None
            for w in range(W):
                u = ps[w] * kv(t, w)
                a = u if a is None else a + u
            outs.append(a * r)
        return outs

    def wo_mm():
        if WS:
            return jnp.concatenate([jax.lax.dot_general(pltpu.bitcast(wot[...], bf16), pltpu.bitcast(o_scr[hh * 64:(hh + 1) * 64, :], bf16), NT,
                                   preferred_element_type=f32) for hh in range(2)], axis=1)
        return jax.lax.dot_general(pltpu.bitcast(wot[...], bf16), pltpu.bitcast(o_scr[...], bf16), NT,
                                   preferred_element_type=f32)

    def zero_from(tok):
        t = pltpu.bitcast(tok, i32)
        return pltpu.bitcast(jnp.minimum(jnp.maximum(t, 0), 0), u32)

    def gate(x, z):
        u = pltpu.bitcast(x, u32)
        k, n = u.shape
        return (u.reshape(k // 8, 8, n) | z[None, :, :n]).reshape(k, n)

    def prep_qkv_t(nb, tok):
        z = zero_from(tok)
        nc = 128 if nb < 13 else 64
        for cb in range(5):
            kc = 128 if cb < 4 else 64
            blk = pltpu.bitcast(gate(wqkv_buf[cb * 128:cb * 128 + kc, nb * 128:nb * 128 + nc], z), bf16)
            t = pltpu.bitcast(blk.T, u32)
            if kc < 128:
                t = jnp.concatenate([t, jnp.zeros((nc // 2, 128 - kc), u32)], axis=1)
            t_scr[cb, nb * 64:nb * 64 + nc // 2, :] = t

    def prep_wo_s(cb, tok):
        z = zero_from(tok)
        kc = 128 if cb < 4 else 64
        t = gate(wo_buf[:, cb * 128:cb * 128 + kc], z)
        if kc < 128:
            t = jnp.concatenate([t, jnp.zeros((D // 2, 128 - kc), u32)], axis=1)
        t2_scr[cb] = t

    def prep_wo_g(kb, tok):
        z = zero_from(tok)
        for cb in range(5):
            kc = 128 if cb < 4 else 64
            g = lambda dp: gate(t2_scr[cb, pl.ds(dp, H, stride=DH // 2), :], z)
            if kb < 4:
                rows = [g(2 * kb), g(2 * kb + 1)]
            else:
                rows = [jnp.zeros((32, 128), u32), g(8)]
            blk = pltpu.bitcast(jnp.concatenate(rows, axis=0), bf16).T
            wot[cb * 64:cb * 64 + kc // 2, kb * 128:(kb + 1) * 128] = pltpu.bitcast(blk[:kc], u32)

    def tk_a(a):
        u = pltpu.bitcast(a, u32)
        return [u[120:128, n * 128:(n + 1) * 128] for n in range(4)]

    def tk_r(r):
        return [r[rows:rows + 8, n * 128:(n + 1) * 128] for n in range(2) for rows in (280, 568)]

    def mm1h(s, hh):
        h = jnp.dot(load_xn(s), w_buf[0, 0, :, hh * 256:(hh + 1) * 256], preferred_element_type=f32) + b1f[0, :, hh * 256:(hh + 1) * 256]
        return mish(h).astype(bf16)

    def ch(hh, k):
        return pltpu.make_async_copy(w1_hbm.at[:, hh * 256:(hh + 1) * 256], w_buf.at[0, 0, :, hh * 256:(hh + 1) * 256], sem.at[k])

    def res(s):
        return x_buf[s].astype(f32)

    cx(0, 0).start(); ch(0, 1).start()
    kv_scr[:, TM:TM + HALO, :] = jnp.zeros((9, HALO, 128), f32)
    cx(0, 0).wait()
    cb1.start(); cx(1, 2).start(); ch(1, 2).start()
    ln(0)
    ch(0, 1).wait(); cb1.wait()
    cw2(0, 0).start(); cx(2, 0).start(); cx(3, 1).start()
    for c in range(NC):
        b1f[c] = b1_buf[c * TF:(c + 1) * TF].astype(f32)[None, :]
    a0a = mm1h(0, 0)
    cx(1, 2).wait(); ch(1, 2).wait()
    cx(4, 1).start(); cx(5, 1).start(); cqkv.start()
    a0b = mm1h(0, 1)
    a0 = jnp.concatenate([a0a, a0b], axis=1)
    ln_c(1, LN1)
    a1 = mm1(0, 1)
    cw2(0, 0).wait(); cx(2, 0).wait()
    cx(6, 2).start(); cx(7, 2).start(); cwo.start()
    acc[0] = mm2(0, a0) + res(0)
    ln_c(2)
    a2 = mm1(0, 2)
    acc[1] = mm2(0, a1) + res(1)
    wx(3, 6, 1)
    cw1(1, 0).start(); cw2(1, 0).start()
    acc[2] = mm2(0, a2) + res(2)
    ln_c(3)
    a3 = mm1(0, 3)
    ln_c(4)
    a4 = mm1(0, 4)
    ln_c(5)
    acc[3] = mm2(0, a3) + res(3)
    cqkv.wait(); wx(6, 8, 2); cwo.wait()
    for c in range(2, NC):
        cw1(c, 1).start(); cw2(c, 1).start()
    a5 = mm1(0, 5)
    ln_c(6)
    tk = tk_a(a5)
    prep_qkv_t(0, tk[2]); prep_qkv_t(1, tk[3])
    r = mm2(0, a4) + res(4)
    acc[4] = r
    tk = tk_r(r)
    ln_c(7, 3, tk[L7T])
    for k in range(4):
        prep_qkv_t(2 + k, tk[k])
    a6 = mm1(0, 6)
    tk = tk_a(a6)
    for k in range(4):
        prep_qkv_t(6 + k, tk[k])
    for cb in range(5):
        prep_wo_s(cb, tk[min(cb, 3)])
    r = mm2(0, a5) + res(5)
    acc[5] = r
    tk = tk_r(r)
    for hh in range(2):
        acc[NS - 1, :, hh * 128:(hh + 1) * 128] = pltpu.bitcast(
            gate(x_buf[NS - 1, :, hh * 128:(hh + 1) * 128], zero_from(tk[2 * hh])), bf16).astype(f32)
    for k in range(4):
        prep_qkv_t(10 + k, tk[k])
    a7 = mm1(0, 7)
    tk = tk_a(a7)
    for kb in range(5):
        prep_wo_g(kb, tk[(0, 0, 1, 2, 3)[kb]])
    acc[6] = mm2(0, a6) + res(6)
    act_last[...] = pltpu.bitcast(a7, u32)
    ww(1, 2, 0)

    def body(cc, carry):
        c = cc
        j = c - 1
        @pl.when(cc == 2)
        def _():
            ww(2, NC, 1)
        acc[NS - 1] = acc[NS - 1] + mm2(c - 1, pltpu.bitcast(act_last[...], bf16))
        qkv_mm(j)
        prev = None
        toks = []
        tnow = 0
        pend = []
        rb_done = 0
        outs = {}
        def run_rb(i, tok):
            outs[i] = attn_rb(j, 8 * i, tok)
            if i % 2 == 1:
                p2 = i // 2
                for t in range(5):
                    o_scr[p2 * 8:(p2 + 1) * 8, t * 128:(t + 1) * 128] = pltpu.bitcast(
                        jnp.concatenate([outs[i - 1][t], outs[i][t]], axis=0).astype(bf16), u32)
        i = 0
        for s in range(NS):
            a = mm1(c, s)
            u = pltpu.bitcast(a, u32)
            for n in SCHED_A[s]:
                run_rb(i, u[120:128, n * 128:(n + 1) * 128]); i += 1
            if prev is not None:
                r = acc[s - 1] + mm2(c, prev)
                acc[s - 1] = r
                out_buf[s - 1] = r.astype(bf16)
                @pl.when(c == NC - 1)
                def _():
                    cout(s - 1).start()
                for n in SCHED_R[s - 1]:
                    rows = (280, 568)[n % 2]
                    run_rb(i, r[rows:rows + 8, (n // 2) * 128:(n // 2 + 1) * 128]); i += 1
            prev = a
        assert i == 32, i
        acc[j] = acc[j] + wo_mm()
        act_last[...] = pltpu.bitcast(prev, u32)
        return carry
    jax.lax.fori_loop(1, NC, body, 0)
    for (r0, r1, hh) in ESPLIT:
        al = pltpu.bitcast(act_last[hh * 64:(hh + 1) * 64, :], bf16)
        r = acc[NS - 1, r0:r1, hh * 128:(hh + 1) * 128] + jax.lax.dot_general(
            w_buf[NC - 1, 1, r0:r1, :], al, NT, preferred_element_type=f32)
        out_buf[NS - 1, r0:r1, hh * 128:(hh + 1) * 128] = r.astype(bf16)
        c0 = (NS - 1) * TM + hh * 128
        pltpu.make_async_copy(out_buf.at[NS - 1, r0:r1, hh * 128:(hh + 1) * 128],
                              out_hbm.at[r0:r1, c0:c0 + 128], sem.at[2]).start()
    pltpu.make_async_copy(out_buf, out_buf, sem.at[2]).wait()


@jax.jit
def pallas_parallel_sum__sliding_local_dilated__dense_activation_mish__prompt_kernel(
        A_x, A_wqkv, A_wo, B_x, B_w1, B_b1, B_w2):
    xt = A_x.reshape(S, D).T
    any_spec = pl.BlockSpec(memory_space=pl.ANY)
    ot = pl.pallas_call(
        kern,
        in_specs=[any_spec] * 6,
        out_specs=any_spec,
        out_shape=jax.ShapeDtypeStruct((D, S), bf16),
        scratch_shapes=[
            pltpu.VMEM((NS, D, TM), bf16),
            pltpu.VMEM((NS, D, TM), bf16),
            pltpu.VMEM((NC, 2, D, TF), bf16),
            pltpu.VMEM((D, 3 * D), bf16),
            pltpu.VMEM((D, D), bf16),
            pltpu.VMEM((F,), bf16),
            pltpu.VMEM((NC, 1, TF), f32),
            pltpu.VMEM((NS, TM // 2, D), u32),
            pltpu.VMEM((NS, 2, 8, TM), f32),
            pltpu.VMEM((NS, D, TM), f32),
            pltpu.VMEM((TM // 2, TF), u32),
            pltpu.VMEM((5, TM, 128), f32),
            pltpu.VMEM((9, TM + HALO, 128), f32),
            pltpu.VMEM((TM // 2, 640), u32),
            pltpu.VMEM((5, 3 * D // 2, 128), u32),
            pltpu.VMEM((5, D // 2, 128), u32),
            pltpu.VMEM((D // 2, 640), u32),
            pltpu.SemaphoreType.DMA((3,)),
        ],
        compiler_params=pltpu.CompilerParams(vmem_limit_bytes=100 * 1024 * 1024),
    )(xt, A_wqkv, A_wo, B_w1, B_b1, B_w2.T)
    return ot.T.reshape(1, S, D)
```

```python
import jax
import jax.numpy as jnp
import numpy as np
import jax.experimental.pallas as pl
import jax.experimental.pallas.tpu as pltpu

S, D, F = 2048, 576, 4608
H, DH, W, DIL = 32, 18, 8, 2
TM, TF = 256, 512
NS, NC = S // TM, F // TF
HALO = 16
NT = (((1,), (1,)), ((), ()))
LOG2E = 1.4426950408889634
QSCALE = (DH ** -0.5) * LOG2E
QBITS = int(np.float32(QSCALE).view(np.int32))
NEG = -1e9 * LOG2E
SCHED_A = [[0, 1, 2, 3], [3], [3], [3], [3], [3], [], []]
SCHED_R = [[0, 1, 2, 3], [0, 1, 2, 3], [0, 1, 2, 3], [0, 1, 2, 3], [0, 1, 2, 3], [0, 1, 2], []]
f32, bf16, u32, i32 = jnp.float32, jnp.bfloat16, jnp.uint32, jnp.int32


def mish(h):
    e = jnp.exp(jnp.minimum(h, 20.0))
    n = e * (e + 2.0)
    return h * (n * pl.reciprocal(n + 2.0, approx=True))


def fold8(a):
    n = a.shape[0] // 8
    parts = [a[8 * i:8 * i + 8] for i in range(n)]
    while len(parts) > 1:
        nxt = [parts[i] + parts[i + 1] for i in range(0, len(parts) - 1, 2)]
        if len(parts) % 2:
            nxt.append(parts[-1])
        parts = nxt
    return parts[0]


def bits_from(tok, bits, dtype):
    t = pltpu.bitcast(tok, i32)
    return pltpu.bitcast(jnp.minimum(jnp.maximum(t, bits), bits), dtype)


def gate(x, z):
    u = pltpu.bitcast(x, u32)
    k, n = u.shape
    return (u.reshape(k // 8, 8, n) | z[None, :, :n]).reshape(k, n)


def kern(x_hbm, wqkv_hbm, wo_hbm, w1_hbm, b1_hbm, w2_hbm, out_hbm,
         x_buf, out_buf, w_buf, wqkv_buf, wo_buf, b1_buf, b1f,
         xn_buf, st_buf, acc, act_last, q_scr, kv_scr, o_scr, t_scr, t2_scr, wot, sem):
    def cx(s, k):
        return pltpu.make_async_copy(x_hbm.at[:, s * TM:(s + 1) * TM], x_buf.at[s], sem.at[k])

    def wx(s0, s1, k):
        pltpu.make_async_copy(x_buf.at[s0:s1], x_buf.at[s0:s1], sem.at[k]).wait()

    def cw1(c, k):
        return pltpu.make_async_copy(w1_hbm.at[:, c * TF:(c + 1) * TF], w_buf.at[c, 0], sem.at[k])

    def cw2(c, k):
        return pltpu.make_async_copy(w2_hbm.at[:, c * TF:(c + 1) * TF], w_buf.at[c, 1], sem.at[k])

    def ww(c0, c1, k):
        pltpu.make_async_copy(w_buf.at[c0:c1], w_buf.at[c0:c1], sem.at[k]).wait()

    def ch(hh, k):
        return pltpu.make_async_copy(w1_hbm.at[:, hh * 256:(hh + 1) * 256],
                                     w_buf.at[0, 0, :, hh * 256:(hh + 1) * 256], sem.at[k])

    cqkv = pltpu.make_async_copy(wqkv_hbm, wqkv_buf, sem.at[2])
    cwo = pltpu.make_async_copy(wo_hbm, wo_buf, sem.at[2])
    cb1 = pltpu.make_async_copy(b1_hbm, b1_buf, sem.at[1])

    def cout(s):
        return pltpu.make_async_copy(out_buf.at[s], out_hbm.at[:, s * TM:(s + 1) * TM], sem.at[2])

    def ln(s):
        tot = None
        for r in range(0, D, 64):
            p = fold8(x_buf[s, r:r + 64, :].astype(f32))
            tot = p if tot is None else tot + p
        m = jnp.sum(tot, axis=0, keepdims=True) * (1.0 / D)
        tot = None
        for r in range(0, D, 96):
            d = x_buf[s, r:r + 96, :].astype(f32) - m
            p = fold8(d * d)
            tot = p if tot is None else tot + p
        v = jnp.sum(tot, axis=0, keepdims=True) * (1.0 / D)
        rs = jax.lax.rsqrt(v + 1e-5)
        st_buf[s, 0] = jnp.broadcast_to(m, (8, TM))
        st_buf[s, 1] = jnp.broadcast_to(rs, (8, TM))
        for r in range(0, D, 128):
            n = min(128, D - r)
            blk = ((x_buf[s, r:r + n, :].astype(f32) - m) * rs).astype(bf16)
            xn_buf[s, :, r:r + n] = pltpu.bitcast(blk.T, u32)

    def ln_c(s, level=3, tok0=None):
        tot = None
        if tok0 is not None:
            z0 = bits_from(tok0, 0, f32)
            tot = jnp.concatenate([z0, z0], axis=1)
        for r in range(0, D, 64):
            blk = x_buf[s, r:r + 64, :].astype(f32)
            for g in range(8):
                p = blk[8 * g:8 * g + 8]
                tot = p if tot is None else tot + p
        m = jnp.broadcast_to(jnp.sum(tot, axis=0, keepdims=True) * (1.0 / D), (8, TM))
        tots = []
        for hh in range(2):
            mh = m[:, hh * 128:(hh + 1) * 128]
            if hh == 1 and level >= 2:
                mh = mh + bits_from(tots[0], 0, f32)
            tot = None
            for r in range(0, D, 96):
                d = x_buf[s, r:r + 96, hh * 128:(hh + 1) * 128].astype(f32).reshape(12, 8, 128) - mh[None]
                dd = d * d
                for g in range(12):
                    tot = dd[g] if tot is None else tot + dd[g]
            tots.append(tot)
        v = jnp.sum(jnp.concatenate(tots, axis=1), axis=0, keepdims=True) * (1.0 / D)
        rs = jnp.broadcast_to(jax.lax.rsqrt(v + 1e-5), (8, TM))
        st_buf[s, 0] = m
        st_buf[s, 1] = rs
        tok = None
        for r in range(0, D, 128):
            n = min(128, D - r)
            mk = m
            if tok is not None and level >= 3:
                z = bits_from(tok, 0, f32)
                mk = m + jnp.concatenate([z, z], axis=1)
            blk = (x_buf[s, r:r + n, :].astype(f32).reshape(n // 8, 8, TM) - mk[None]) * rs[None]
            blk = blk.reshape(n, TM).astype(bf16)
            t = pltpu.bitcast(blk.T, u32)
            xn_buf[s, :, r:r + n] = t
            if n == 128:
                tok = t[0:8, :]

    def load_xn(s):
        return pltpu.bitcast(xn_buf[s], bf16)

    def res(s):
        return x_buf[s].astype(f32)

    def mm1(c, s):
        outs = []
        for n0 in range(0, TF, 128):
            h = jnp.dot(load_xn(s), w_buf[c, 0, :, n0:n0 + 128], preferred_element_type=f32) + b1f[c, :, n0:n0 + 128]
            outs.append(mish(h).astype(bf16))
        return jnp.concatenate(outs, axis=1)

    def mm1h(s, hh):
        h = (jnp.dot(load_xn(s), w_buf[0, 0, :, hh * 256:(hh + 1) * 256], preferred_element_type=f32)
             + b1f[0, :, hh * 256:(hh + 1) * 256])
        return mish(h).astype(bf16)

    def mm2(c, a):
        return jax.lax.dot_general(w_buf[c, 1], a, NT, preferred_element_type=f32)

    def tk_a(a):
        u = pltpu.bitcast(a, u32)
        return [u[120:128, n * 128:(n + 1) * 128] for n in range(4)]

    def tk_r(r):
        return [r[rows:rows + 8, n * 128:(n + 1) * 128] for n in range(2) for rows in (280, 568)]

    def qkv_mm(j):
        kv_scr[:, 0:HALO, :] = kv_scr[:, TM:TM + HALO, :]
        xnt = ((x_buf[j].astype(f32).reshape(D // 8, 8, TM) - st_buf[j, 0][None]) * st_buf[j, 1][None]
               ).reshape(D, TM).astype(bf16)
        tails = []
        for t in (1, 2, 0):
            cols = []
            for cb in range(5):
                col = jnp.concatenate([t_scr[cb, pl.ds(t * (D // 2) + dp, H, stride=DH // 2), :]
                                       for dp in range(DH // 2)], axis=0)
                cols.append(col if cb < 4 else col[:, :64])
            wblk = pltpu.bitcast(jnp.concatenate(cols, axis=1), bf16)
            r = jnp.dot(wblk, xnt, preferred_element_type=f32)
            for g in range(4):
                blk = r[g * 128:(g + 1) * 128].T
                if t == 0:
                    q_scr[g] = blk
                else:
                    kv_scr[(t - 1) * 4 + g, HALO:HALO + TM, :] = blk
            if t == 0:
                q_scr[4] = jnp.concatenate([r[512:576], jnp.zeros((64, TM), f32)], axis=0).T
            else:
                tails.append(r[512:576])
        kv_scr[8, HALO:HALO + TM, :] = jnp.concatenate(tails, axis=0).T

    def attn_rb(j, r0, tok):
        sc = bits_from(tok, QBITS, f32)
        odd = (jax.lax.broadcasted_iota(jnp.int32, (8, 128), 1) & 1) == 1
        q = [q_scr[t, r0:r0 + 8, :] * sc for t in range(5)]

        def kv(t, w):
            return kv_scr[t, pl.ds(HALO + r0 - DIL * w, 8), :]
        ls = []
        for w in range(W):
            p = q[0] * kv(0, w)
            for t in range(1, 4):
                p = p + q[t] * kv(t, w)
            p = p + q[4] * kv(8, w)
            p = p + pltpu.roll(p, 64, 1)
            p = p + jnp.where(odd, pltpu.roll(p, 1, 1), pltpu.roll(p, 127, 1))
            if r0 < 16 and w > 0:
                pos = j * TM + r0 + jax.lax.broadcasted_iota(jnp.int32, (8, 128), 0)
                p = jnp.where(pos >= DIL * w, p, NEG)
            ls.append(p)
        mx = jnp.maximum(jnp.maximum(jnp.maximum(ls[0], ls[1]), jnp.maximum(ls[2], ls[3])),
                         jnp.maximum(jnp.maximum(ls[4], ls[5]), jnp.maximum(ls[6], ls[7])))
        ps = [jnp.exp2(l - mx) for l in ls]
        den = ((ps[0] + ps[1]) + (ps[2] + ps[3])) + ((ps[4] + ps[5]) + (ps[6] + ps[7]))
        r = pl.reciprocal(den, approx=True)
        outs = []
        for t in (4, 5, 6, 7, 8):
            a = None
            for w in range(W):
                u = ps[w] * kv(t, w)
                a = u if a is None else a + u
            outs.append(a * r)
        return outs

    def wo_mm():
        return jax.lax.dot_general(pltpu.bitcast(wot[...], bf16), pltpu.bitcast(o_scr[...], bf16), NT,
                                   preferred_element_type=f32)

    def prep_qkv_t(nb, tok):
        z = bits_from(tok, 0, u32)
        nc = 128 if nb < 13 else 64
        for cb in range(5):
            kc = 128 if cb < 4 else 64
            blk = pltpu.bitcast(gate(wqkv_buf[cb * 128:cb * 128 + kc, nb * 128:nb * 128 + nc], z), bf16)
            t = pltpu.bitcast(blk.T, u32)
            if kc < 128:
                t = jnp.concatenate([t, jnp.zeros((nc // 2, 128 - kc), u32)], axis=1)
            t_scr[cb, nb * 64:nb * 64 + nc // 2, :] = t

    def prep_wo_s(cb, tok):
        z = bits_from(tok, 0, u32)
        kc = 128 if cb < 4 else 64
        t = gate(wo_buf[:, cb * 128:cb * 128 + kc], z)
        if kc < 128:
            t = jnp.concatenate([t, jnp.zeros((D // 2, 128 - kc), u32)], axis=1)
        t2_scr[cb] = t

    def prep_wo_g(kb, tok):
        z = bits_from(tok, 0, u32)
        for cb in range(5):
            kc = 128 if cb < 4 else 64
            g = lambda dp: gate(t2_scr[cb, pl.ds(dp, H, stride=DH // 2), :], z)
            if kb < 4:
                rows = [g(2 * kb), g(2 * kb + 1)]
            else:
                rows = [jnp.zeros((32, 128), u32), g(8)]
            blk = pltpu.bitcast(jnp.concatenate(rows, axis=0), bf16).T
            wot[cb * 64:cb * 64 + kc // 2, kb * 128:(kb + 1) * 128] = pltpu.bitcast(blk[:kc], u32)

    cx(0, 0).start(); ch(0, 1).start()
    kv_scr[:, TM:TM + HALO, :] = jnp.zeros((9, HALO, 128), f32)
    cx(0, 0).wait()
    cb1.start(); cx(1, 2).start(); ch(1, 2).start()
    ln(0)
    ch(0, 1).wait(); cb1.wait()
    cw2(0, 0).start(); cx(2, 0).start(); cx(3, 1).start()
    for c in range(NC):
        b1f[c] = b1_buf[c * TF:(c + 1) * TF].astype(f32)[None, :]
    a0a = mm1h(0, 0)
    cx(1, 2).wait(); ch(1, 2).wait()
    cx(4, 1).start(); cx(5, 1).start(); cqkv.start()
    a0b = mm1h(0, 1)
    a0 = jnp.concatenate([a0a, a0b], axis=1)
    ln_c(1, 2)
    a1 = mm1(0, 1)
    cw2(0, 0).wait(); cx(2, 0).wait()
    cx(6, 2).start(); cx(7, 2).start(); cwo.start()
    acc[0] = mm2(0, a0) + res(0)
    ln_c(2)
    a2 = mm1(0, 2)
    acc[1] = mm2(0, a1) + res(1)
    wx(3, 6, 1)
    cw1(1, 0).start(); cw2(1, 0).start()
    acc[2] = mm2(0, a2) + res(2)
    ln_c(3)
    a3 = mm1(0, 3)
    ln_c(4)
    a4 = mm1(0, 4)
    ln_c(5)
    acc[3] = mm2(0, a3) + res(3)
    cqkv.wait(); wx(6, 8, 2); cwo.wait()
    for c in range(2, NC):
        cw1(c, 1).start(); cw2(c, 1).start()
    a5 = mm1(0, 5)
    ln_c(6)
    tk = tk_a(a5)
    prep_qkv_t(0, tk[2]); prep_qkv_t(1, tk[3])
    r = mm2(0, a4) + res(4)
    acc[4] = r
    tk = tk_r(r)
    ln_c(7, 3, tk[0])
    for k in range(4):
        prep_qkv_t(2 + k, tk[k])
    a6 = mm1(0, 6)
    tk = tk_a(a6)
    for k in range(4):
        prep_qkv_t(6 + k, tk[k])
    for cb in range(5):
        prep_wo_s(cb, tk[min(cb, 3)])
    r = mm2(0, a5) + res(5)
    acc[5] = r
    tk = tk_r(r)
    for hh in range(2):
        acc[NS - 1, :, hh * 128:(hh + 1) * 128] = pltpu.bitcast(
            gate(x_buf[NS - 1, :, hh * 128:(hh + 1) * 128], bits_from(tk[2 * hh], 0, u32)), bf16).astype(f32)
    for k in range(4):
        prep_qkv_t(10 + k, tk[k])
    a7 = mm1(0, 7)
    tk = tk_a(a7)
    for kb in range(5):
        prep_wo_g(kb, tk[(0, 0, 1, 2, 3)[kb]])
    acc[6] = mm2(0, a6) + res(6)
    act_last[...] = pltpu.bitcast(a7, u32)
    ww(1, 2, 0)

    def body(c, carry):
        j = c - 1

        @pl.when(c == 2)
        def _():
            ww(2, NC, 1)

        acc[NS - 1] = acc[NS - 1] + mm2(c - 1, pltpu.bitcast(act_last[...], bf16))
        qkv_mm(j)
        outs = {}

        def run_rb(i, tok):
            outs[i] = attn_rb(j, 8 * i, tok)
            if i % 2 == 1:
                p2 = i // 2
                for t in range(5):
                    o_scr[p2 * 8:(p2 + 1) * 8, t * 128:(t + 1) * 128] = pltpu.bitcast(
                        jnp.concatenate([outs[i - 1][t], outs[i][t]], axis=0).astype(bf16), u32)
        prev = None
        i = 0
        for s in range(NS):
            a = mm1(c, s)
            u = pltpu.bitcast(a, u32)
            for n in SCHED_A[s]:
                run_rb(i, u[120:128, n * 128:(n + 1) * 128]); i += 1
            if prev is not None:
                r = acc[s - 1] + mm2(c, prev)
                acc[s - 1] = r
                out_buf[s - 1] = r.astype(bf16)

                @pl.when(c == NC - 1)
                def _():
                    cout(s - 1).start()

                for n in SCHED_R[s - 1]:
                    rows = (280, 568)[n % 2]
                    run_rb(i, r[rows:rows + 8, (n // 2) * 128:(n // 2 + 1) * 128]); i += 1
            prev = a
        assert i == 32
        acc[j] = acc[j] + wo_mm()
        act_last[...] = pltpu.bitcast(prev, u32)
        return carry

    jax.lax.fori_loop(1, NC, body, 0)

    for (r0, r1, hh) in [(0, D, 0), (0, 288, 1), (288, D, 1)]:
        al = pltpu.bitcast(act_last[hh * 64:(hh + 1) * 64, :], bf16)
        r = acc[NS - 1, r0:r1, hh * 128:(hh + 1) * 128] + jax.lax.dot_general(
            w_buf[NC - 1, 1, r0:r1, :], al, NT, preferred_element_type=f32)
        out_buf[NS - 1, r0:r1, hh * 128:(hh + 1) * 128] = r.astype(bf16)
        c0 = (NS - 1) * TM + hh * 128
        pltpu.make_async_copy(out_buf.at[NS - 1, r0:r1, hh * 128:(hh + 1) * 128],
                              out_hbm.at[r0:r1, c0:c0 + 128], sem.at[2]).start()
    pltpu.make_async_copy(out_buf, out_buf, sem.at[2]).wait()


@jax.jit
def pallas_parallel_sum__sliding_local_dilated__dense_activation_mish__prompt_kernel(
        A_x, A_wqkv, A_wo, B_x, B_w1, B_b1, B_w2):
    xt = A_x.reshape(S, D).T
    any_spec = pl.BlockSpec(memory_space=pl.ANY)
    ot = pl.pallas_call(
        kern,
        in_specs=[any_spec] * 6,
        out_specs=any_spec,
        out_shape=jax.ShapeDtypeStruct((D, S), bf16),
        scratch_shapes=[
            pltpu.VMEM((NS, D, TM), bf16),
            pltpu.VMEM((NS, D, TM), bf16),
            pltpu.VMEM((NC, 2, D, TF), bf16),
            pltpu.VMEM((D, 3 * D), bf16),
            pltpu.VMEM((D, D), bf16),
            pltpu.VMEM((F,), bf16),
            pltpu.VMEM((NC, 1, TF), f32),
            pltpu.VMEM((NS, TM // 2, D), u32),
            pltpu.VMEM((NS, 2, 8, TM), f32),
            pltpu.VMEM((NS, D, TM), f32),
            pltpu.VMEM((TM // 2, TF), u32),
            pltpu.VMEM((5, TM, 128), f32),
            pltpu.VMEM((9, TM + HALO, 128), f32),
            pltpu.VMEM((TM // 2, 640), u32),
            pltpu.VMEM((5, 3 * D // 2, 128), u32),
            pltpu.VMEM((5, D // 2, 128), u32),
            pltpu.VMEM((D // 2, 640), u32),
            pltpu.SemaphoreType.DMA((3,)),
        ],
        compiler_params=pltpu.CompilerParams(vmem_limit_bytes=100 * 1024 * 1024),
    )(xt, A_wqkv, A_wo, B_w1, B_b1, B_w2.T)
    return ot.T.reshape(1, S, D)
```
